```python
import jax
import jax.numpy as jnp

def _softmax(x, axis=-1):
    return jax.nn.softmax(x, axis=axis)
def _gelu(x):
    return jax.nn.gelu(x, approximate=True)
def _silu(x):
    return jax.nn.silu(x)
def _sigmoid(x):
    return jax.nn.sigmoid(x)
def _layernorm(x, axis=-1, eps=1e-5):
    m = jnp.mean(x, axis=axis, keepdims=True)
    v = jnp.var(x, axis=axis, keepdims=True)
    return (x - m) / jnp.sqrt(v + eps)
def _scatter_add(tgt, idx, src, axis=0):
    return tgt.at[idx].add(src)
def _segment_sum(src, seg, n):
    return jax.ops.segment_sum(src, seg, n)
class _Rng:
    def __init__(self, key):
        self._k = key
    def _next(self):
        self._k, sub = jax.random.split(self._k)
        return sub
    def normal(self, shape):
        return jax.random.normal(self._next(), shape, dtype=jnp.bfloat16)
    def randint(self, lo, hi, shape):
        return jax.random.randint(self._next(), shape, lo, hi, dtype=jnp.int32)
    def uniform(self, shape, lo=0.0, hi=1.0):
        return jax.random.uniform(self._next(), shape, jnp.bfloat16, lo, hi)
    def permutation(self, n):
        return jax.random.permutation(self._next(), n)


kernel_name = 'concat_heads__mha_block_cached__compressed_kv_cla__decode'

def setup_inputs():
    _rng = _Rng(jax.random.key(int.from_bytes(__import__("os").urandom(4), "little")))
    _w = (lambda a: (lambda t: t.astype(jnp.bfloat16) if jnp.issubdtype(t.dtype, jnp.floating) else t)(jnp.asarray(a)))
    def _A_setup():
        B, Sq, D = 4, 1, 576
        H, Sk, Dh = 32, 4096, 128
        return {
            "x": _w((lambda *s: _rng.normal(s) * 0.05)(B, Sq, D)),
            "k_cache": _w((lambda *s: _rng.normal(s) * 0.05)(B, H, Sk, Dh)),
            "v_cache": _w((lambda *s: _rng.normal(s) * 0.05)(B, H, Sk, Dh)),
            "wq": _w((lambda *s: _rng.normal(s) * 0.05)(D, H * Dh) * (D ** -0.5)),
            "wo": _w((lambda *s: _rng.normal(s) * 0.05)(H * Dh, D) * ((H * Dh) ** -0.5)),
        }
    _A_in = _A_setup()

    def _B_setup():
        B, H, Sq, Sk, D, M = 4, 32, 1, 4096, 128, 576
        Dc = 4 * D
        return {
            "x": _w((lambda *s: _rng.normal(s) * 0.05)(B, Sq, M)),
            "c_kv": _w((lambda *s: _rng.normal(s) * 0.05)(B, Sk, Dc)),
            "w_q": _w((lambda *s: _rng.normal(s) * 0.05)(M, H, D) * (M ** -0.5)),
            "w_uk": _w((lambda *s: _rng.normal(s) * 0.05)(Dc, H, D) * (Dc ** -0.5)),
            "w_uv": _w((lambda *s: _rng.normal(s) * 0.05)(Dc, H, D) * (Dc ** -0.5)),
            "w_o": _w((lambda *s: _rng.normal(s) * 0.05)(H, D, M) * ((H * D) ** -0.5)),
        }
    _B_in = _B_setup()

    return {
        "A_x": _A_in["x"],
        "A_k_cache": _A_in["k_cache"],
        "A_v_cache": _A_in["v_cache"],
        "A_wq": _A_in["wq"],
        "A_wo": _A_in["wo"],
        "B_x": _B_in["x"],
        "B_c_kv": _B_in["c_kv"],
        "B_w_q": _B_in["w_q"],
        "B_w_uk": _B_in["w_uk"],
        "B_w_uv": _B_in["w_uv"],
        "B_w_o": _B_in["w_o"],
    }

def reference(A_x, A_k_cache, A_v_cache, A_wq, A_wo, B_x, B_c_kv, B_w_q, B_w_uk, B_w_uv, B_w_o):
    def _A_ref(x, k_cache, v_cache, wq, wo):
        B, Sq, D = x.shape
        H, Dh = 32, 128
        q = (lambda x, *d: x.transpose(*d))((x @ wq).reshape(B, Sq, H, Dh), 0, 2, 1, 3)
        scores = jnp.einsum("bhqd,bhkd->bhqk", q, k_cache) * (Dh ** -0.5)
        p = _softmax(scores, axis=-1)
        o = jnp.einsum("bhqk,bhkd->bhqd", p, v_cache)
        return (lambda x, *d: x.transpose(*d))(o, 0, 2, 1, 3).reshape(B, Sq, H * Dh) @ wo

    def _B_ref(x, c_kv, w_q, w_uk, w_uv, w_o):
        B, Sq, M = x.shape[0], x.shape[1], x.shape[2]
        Sk = c_kv.shape[1]
        H, D = w_q.shape[1], w_q.shape[2]
        q = jnp.einsum("bqm,mhd->bhqd", x, w_q)
        k = jnp.einsum("bkc,chd->bhkd", c_kv, w_uk)
        v = jnp.einsum("bkc,chd->bhkd", c_kv, w_uv)
        scores = jnp.einsum("bhqd,bhkd->bhqk", q, k) * (D ** -0.5)
        off = Sk - Sq
        qi = jnp.arange(Sq)[:, None]
        kj = jnp.arange(Sk)[None, :]
        cmask = kj <= (qi + off)
        scores = jnp.where(cmask[None, None], scores, -1e9)
        p = _softmax(scores, axis=-1)
        ctx = jnp.einsum("bhqk,bhkd->bhqd", p, v)
        return jnp.einsum("bhqd,hdm->bqm", ctx, w_o)

    a = _A_ref(A_x, A_k_cache, A_v_cache, A_wq, A_wo)
    b = _B_ref(B_x, B_c_kv, B_w_q, B_w_uk, B_w_uv, B_w_o)
    return jnp.concatenate([a, b], axis=-1)
```

```python
import functools

import jax
import jax.numpy as jnp
from jax import lax
from jax.experimental import pallas as pl
from jax.experimental.pallas import tpu as pltpu

B = 4
H = 32
S = 4096
D = 128
M = 576
C = 512
SCALE = D ** -0.5

KV_ROWS = 192
NBUF = 3
W_ROWS = 192
X_CHUNK = 6
C_ROWS = 48

BF16 = jnp.bfloat16
F32 = jnp.float32

_NT = (((1,), (1,)), ((), ()))


def _chunked(total, size, fn):
    n_full = total // size

    def body(c, carry):
        fn(pl.multiple_of(c * size, 8 if size % 8 == 0 else 1), size)
        return carry

    lax.fori_loop(0, n_full, body, 0)
    if total % size:
        fn(n_full * size, total % size)


def _kernel(xa_hbm, k_hbm, v_hbm, wq_hbm, wot_hbm,
            xb_hbm, c_hbm, wqb_hbm, wuk_hbm, wuv_hbm, wobt_hbm,
            out_ref,
            xa_v, xb_v, wq_v, wot_v, wqb_v, wuk_v, wuv_v, wobt_v, c_v,
            kbuf, vbuf,
            acc_a, qb_s, qa_s, qat_s, p_s, l_s, cc_s, ctx_s, outb_s,
            kv_sem, w_sem):
    copy = pltpu.make_async_copy

    def wait_buf(buf, sem):
        copy(buf, buf, sem).wait()

    def issue_kv(step, slot):
        h = step // B
        b = step % B

        def fn(r0, n):
            copy(k_hbm.at[b, h, pl.ds(r0, n)], kbuf.at[slot, pl.ds(r0, n)],
                 kv_sem.at[0, slot]).start(priority=0)
            copy(v_hbm.at[b, h, pl.ds(r0, n)], vbuf.at[slot, pl.ds(r0, n)],
                 kv_sem.at[1, slot]).start(priority=1)

        _chunked(S, KV_ROWS, fn)

    copy(xa_hbm, xa_v, w_sem.at[0]).start(priority=0)
    copy(xb_hbm, xb_v, w_sem.at[1]).start(priority=1)

    n_sub = M // W_ROWS

    def head_blocks(src2d, dst3d, sem, src3d, x3d_dst, sem2, second_is_headblock):
        def body(t, carry):
            h = t // n_sub
            r0 = pl.multiple_of((t % n_sub) * W_ROWS, 8)
            c0 = pl.multiple_of(h * D, D)
            copy(src2d.at[pl.ds(r0, W_ROWS), pl.ds(c0, D)],
                 dst3d.at[h, pl.ds(r0, W_ROWS)], sem).start(priority=0)
            if second_is_headblock:
                copy(src3d.at[h, pl.ds(r0, W_ROWS)],
                     x3d_dst.at[h, pl.ds(r0, W_ROWS)], sem2).start(priority=1)
            else:
                m0 = t * X_CHUNK
                copy(src3d.at[pl.ds(m0, X_CHUNK)],
                     x3d_dst.at[pl.ds(m0, X_CHUNK)], sem2).start(priority=1)
            return carry

        lax.fori_loop(0, H * n_sub, body, 0)

    head_blocks(wq_hbm, wq_v, w_sem.at[2], wqb_hbm, wqb_v, w_sem.at[3], False)
    head_blocks(wot_hbm, wot_v, w_sem.at[4], wobt_hbm, wobt_v, w_sem.at[5], True)

    def uk_uv(r0, n):
        copy(wuk_hbm.at[pl.ds(r0, n)], wuk_v.at[pl.ds(r0, n)], w_sem.at[6]).start(priority=0)
        copy(wuv_hbm.at[pl.ds(r0, n)], wuv_v.at[pl.ds(r0, n)], w_sem.at[7]).start(priority=1)

    _chunked(C, X_CHUNK, uk_uv)

    for b0 in (0, 2):
        def ckv(r0, n, b0=b0):
            copy(c_hbm.at[b0, pl.ds(r0, n)], c_v.at[b0, pl.ds(r0, n)],
                 w_sem.at[8 + b0]).start(priority=0)
            copy(c_hbm.at[b0 + 1, pl.ds(r0, n)], c_v.at[b0 + 1, pl.ds(r0, n)],
                 w_sem.at[9 + b0]).start(priority=1)

        _chunked(S, C_ROWS, ckv)

    for j in range(NBUF):
        issue_kv(j, j)

    wait_buf(xa_v, w_sem.at[0])
    wait_buf(wq_v, w_sem.at[2])
    wait_buf(wot_v, w_sem.at[4])
    acc_a[...] = jnp.zeros(acc_a.shape, F32)

    def b_q(m_lo, m_hi, first):
        def run():
            if first:
                wait_buf(xb_v, w_sem.at[1])
                wait_buf(wqb_v, w_sem.at[3])
            wt = jnp.swapaxes(wqb_v[m_lo:m_hi], 0, 1)
            x = xb_v[:, m_lo:m_hi]
            for h in range(H):
                r = jnp.dot(x, wt[h], preferred_element_type=F32)
                if first:
                    qb_s[h] = r
                else:
                    qb_s[h] = qb_s[h] + r
        return run

    def b_qabs(c_lo, c_hi, first):
        def run():
            if first:
                wait_buf(wuk_v, w_sem.at[6])
            wt = jnp.swapaxes(wuk_v[c_lo:c_hi], 0, 1)
            for h in range(H):
                qa_s[h, :, c_lo:c_hi] = lax.dot_general(
                    qb_s[h].astype(BF16), wt[h], _NT, preferred_element_type=F32)
        return run

    def b_qabs_t():
        qat_s[...] = jnp.swapaxes(qa_s[...], 0, 1).astype(BF16)

    def b_scores(b):
        def run():
            wait_buf(c_v.at[b], w_sem.at[8 + b])
            s = lax.dot_general(qat_s[b], c_v[b], _NT, preferred_element_type=F32)
            m = jnp.max(s, axis=-1, keepdims=True)
            p = jnp.exp((s - m) * SCALE)
            l_s[b] = jnp.broadcast_to(jnp.sum(p, axis=-1, keepdims=True), (H, D))
            p_s[...] = p.astype(BF16)
        return run

    def b_pv(b):
        def run():
            cc = jnp.dot(p_s[...], c_v[b], preferred_element_type=F32)
            cc_s[b] = cc / l_s[b][:, 0:1]
        return run

    def b_ctx(c_lo, c_hi, first):
        def run():
            if first:
                wait_buf(wuv_v, w_sem.at[7])
            wt = jnp.swapaxes(wuv_v[c_lo:c_hi], 0, 1)
            cct = jnp.swapaxes(cc_s[:, :, c_lo:c_hi], 0, 1).astype(BF16)
            for h in range(H):
                r = jnp.dot(cct[h], wt[h], preferred_element_type=F32)
                if first:
                    ctx_s[h] = r
                else:
                    ctx_s[h] = ctx_s[h] + r
        return run

    def b_out():
        wait_buf(wobt_v, w_sem.at[5])
        o = jnp.zeros((B, M), F32)
        for h in range(H):
            o = o + lax.dot_general(ctx_s[h].astype(BF16), wobt_v[h], _NT,
                                    preferred_element_type=F32)
        outb_s[...] = o

    pieces = [b_q(0, 256, True), b_q(256, 576, False),
              b_qabs(0, 256, True), b_qabs(256, 512, False), b_qabs_t]
    for b in range(B):
        pieces += [b_scores(b), b_pv(b)]
    pieces += [b_ctx(0, 256, True), b_ctx(256, 512, False), b_out]

    def step(i, carry):
        slot = i % NBUF
        h = i // B
        b = i % B
        q = jnp.dot(xa_v[...], wq_v[h], preferred_element_type=F32).astype(BF16)
        wait_buf(kbuf.at[slot], kv_sem.at[0, slot])
        s = lax.dot_general(q, kbuf[slot], _NT, preferred_element_type=F32)
        m = jnp.max(s, axis=-1, keepdims=True)
        p = jnp.exp((s - m) * SCALE)
        l = jnp.sum(p, axis=-1, keepdims=True)
        wait_buf(vbuf.at[slot], kv_sem.at[1, slot])
        o = jnp.dot(p.astype(BF16), vbuf[slot], preferred_element_type=F32)
        row = lax.broadcasted_iota(jnp.int32, (B, D), 0)
        o = jnp.where(row == b, o / l, 0.0).astype(BF16)
        acc_a[...] += lax.dot_general(o, wot_v[h], _NT, preferred_element_type=F32)

        for n, piece in enumerate(pieces):
            pl.when(i == n + 1)(piece)

        @pl.when(i + NBUF < B * H)
        def _():
            issue_kv(i + NBUF, slot)

        return carry

    lax.fori_loop(0, B * H, step, 0)

    out_ref[:, 0:M] = acc_a[...].astype(out_ref.dtype)
    out_ref[:, M:2 * M] = outb_s[...].astype(out_ref.dtype)


@jax.jit
def pallas_concat_heads__mha_block_cached__compressed_kv_cla__decode_kernel(
    A_x: jax.Array,
    A_k_cache: jax.Array,
    A_v_cache: jax.Array,
    A_wq: jax.Array,
    A_wo: jax.Array,
    B_x: jax.Array,
    B_c_kv: jax.Array,
    B_w_q: jax.Array,
    B_w_uk: jax.Array,
    B_w_uv: jax.Array,
    B_w_o: jax.Array,
):
    xa = A_x.reshape(B, M)
    xb = B_x.reshape(B, M)
    wot = A_wo.T
    wobt = B_w_o.transpose(0, 2, 1)

    hbm = pl.BlockSpec(memory_space=pl.ANY)
    scratch = [
        pltpu.VMEM((B, M), BF16),
        pltpu.VMEM((B, M), BF16),
        pltpu.VMEM((H, M, D), BF16),
        pltpu.VMEM((H, M, D), BF16),
        pltpu.VMEM((M, H, D), BF16),
        pltpu.VMEM((C, H, D), BF16),
        pltpu.VMEM((C, H, D), BF16),
        pltpu.VMEM((H, M, D), BF16),
        pltpu.VMEM((B, S, C), BF16),
        pltpu.VMEM((NBUF, S, D), BF16),
        pltpu.VMEM((NBUF, S, D), BF16),
        pltpu.VMEM((B, M), F32),
        pltpu.VMEM((H, B, D), F32),
        pltpu.VMEM((H, B, C), F32),
        pltpu.VMEM((B, H, C), BF16),
        pltpu.VMEM((H, S), BF16),
        pltpu.VMEM((B, H, D), F32),
        pltpu.VMEM((B, H, C), F32),
        pltpu.VMEM((H, B, D), F32),
        pltpu.VMEM((B, M), F32),
        pltpu.SemaphoreType.DMA((2, NBUF)),
        pltpu.SemaphoreType.DMA((12,)),
    ]
    out = pl.pallas_call(
        _kernel,
        out_shape=jax.ShapeDtypeStruct((B, 2 * M), BF16),
        in_specs=[hbm] * 11,
        out_specs=pl.BlockSpec(memory_space=pltpu.VMEM),
        scratch_shapes=scratch,
        compiler_params=pltpu.CompilerParams(vmem_limit_bytes=100 * 1024 * 1024),
    )(xa, A_k_cache, A_v_cache, A_wq, wot, xb, B_c_kv, B_w_q, B_w_uk, B_w_uv, wobt)
    return out.reshape(B, 1, 2 * M)
```

```python
import jax
import jax.numpy as jnp
from jax import lax
from jax.experimental import pallas as pl
from jax.experimental.pallas import tpu as pltpu

B = 4
H = 32
S = 4096
D = 128
M = 576
C = 512
SCALE = D ** -0.5
NSTEP = B * H

K_CHUNKS = [128] + [192] * 20 + [128]
V_CHUNKS = [112] + [192] * 20 + [144]
NBUF = 4
WA_COLS = 2048
W_ROWS = 192
X_CHUNK = 6
C_ROWS = 48
DEFER = 4
PIECE_START = 1
PIECE_STRIDE = 4

BF16 = jnp.bfloat16
F32 = jnp.float32

_NT = (((1,), (1,)), ((), ()))


def _spans(sizes):
    assert sum(sizes) == S
    out, start = [], 0
    for n in sizes:
        out.append((start, n))
        start += n
    return out


_KV_ORDER = sorted([(r0 + n / 2, 0, r0, n) for r0, n in _spans(K_CHUNKS)]
                   + [(r0 + n / 2 + 0.1, 1, r0, n) for r0, n in _spans(V_CHUNKS)])


def _chunked(total, size, fn):
    n_full = total // size

    def body(c, carry):
        fn(pl.multiple_of(c * size, 8 if size % 8 == 0 else 1), size)
        return carry

    lax.fori_loop(0, n_full, body, 0)
    if total % size:
        fn(n_full * size, total % size)


def _kernel(xa_hbm, k_hbm, v_hbm, wq_hbm, wot_hbm,
            xb_hbm, c_hbm, wqb_hbm, wuk_hbm, wuv_hbm, wobt_hbm,
            out_hbm,
            xa_v, xb_v, wq_v, wot_v, wqb_v, wuk_v, wuv_v, wobt_v, c_v,
            kbuf, vbuf,
            acc_a, pa_s, la_s, qb_s, qa_s, qat_s, p_s, l_s, cc_s, ctx_s, outb_s, out_v,
            kv_sem, w_sem, d_sem):
    copy = pltpu.make_async_copy
    n_sub = M // W_ROWS
    n_early = H - DEFER

    def wait_buf(buf, sem):
        copy(buf, buf, sem).wait()

    def head_cols(ref, h):
        return ref[:, pl.ds(pl.multiple_of(h * D, D), D)]

    def issue_kv(step, slot):
        b = step // H
        h = step % H
        for _, is_v, r0, n in _KV_ORDER:
            src, dst = (v_hbm, vbuf) if is_v else (k_hbm, kbuf)
            copy(src.at[b, h, pl.ds(r0, n)], dst.at[slot, pl.ds(r0, n)],
                 kv_sem.at[is_v, slot]).start(priority=is_v)

    copy(xa_hbm, xa_v, w_sem.at[0]).start(priority=0)
    copy(xb_hbm, xb_v, w_sem.at[1]).start(priority=1)

    n_col = (H * D) // WA_COLS

    def wa_body(t, carry):
        idx = (pl.ds(pl.multiple_of((t // n_col) * 8, 8), 8),
               pl.ds(pl.multiple_of((t % n_col) * WA_COLS, D), WA_COLS))
        copy(wq_hbm.at[idx], wq_v.at[idx], w_sem.at[2]).start(priority=0)
        copy(wot_hbm.at[idx], wot_v.at[idx], w_sem.at[4]).start(priority=1)
        return carry

    lax.fori_loop(0, (M // 8) * n_col, wa_body, 0)

    xc = M // (H * n_sub)

    def wqb_chunk(t):
        copy(wqb_hbm.at[pl.ds(t * xc, xc)], wqb_v.at[pl.ds(t * xc, xc)],
             w_sem.at[3]).start(priority=0)

    def wb_body(t, carry):
        wqb_chunk(t)
        h = t // n_sub
        r0 = pl.multiple_of((t % n_sub) * W_ROWS, 8)
        copy(wobt_hbm.at[h, pl.ds(r0, W_ROWS)], wobt_v.at[h, pl.ds(r0, W_ROWS)],
             w_sem.at[5]).start(priority=1)
        return carry

    lax.fori_loop(0, n_early * n_sub, wb_body, 0)

    def wb_tail(t, carry):
        wqb_chunk(t)
        return carry

    lax.fori_loop(n_early * n_sub, H * n_sub, wb_tail, 0)

    def uk_uv(r0, n):
        copy(wuk_hbm.at[pl.ds(r0, n)], wuk_v.at[pl.ds(r0, n)], w_sem.at[6]).start(priority=0)
        copy(wuv_hbm.at[pl.ds(r0, n)], wuv_v.at[pl.ds(r0, n)], w_sem.at[7]).start(priority=1)

    _chunked(C, X_CHUNK, uk_uv)

    for b0 in (0, 2):
        def ckv(r0, n, b0=b0):
            copy(c_hbm.at[b0, pl.ds(r0, n)], c_v.at[b0, pl.ds(r0, n)],
                 w_sem.at[8 + b0]).start(priority=0)
            copy(c_hbm.at[b0 + 1, pl.ds(r0, n)], c_v.at[b0 + 1, pl.ds(r0, n)],
                 w_sem.at[9 + b0]).start(priority=1)

        _chunked(S, C_ROWS, ckv)

    for j in range(NBUF):
        issue_kv(j, j)

    def issue_deferred():
        for j in range(DEFER):
            h = n_early + j
            sem = d_sem.at[0 if j < DEFER - 1 else 1]
            for t in range(n_sub):
                copy(wobt_hbm.at[h, pl.ds(t * W_ROWS, W_ROWS)],
                     wobt_v.at[h, pl.ds(t * W_ROWS, W_ROWS)], sem).start(priority=1)

    def k_phase(j):
        slot = j % NBUF
        h = j % H
        q = jnp.dot(xa_v[...], head_cols(wq_v, h),
                    preferred_element_type=F32).astype(BF16)
        wait_buf(kbuf.at[slot], kv_sem.at[0, slot])
        s = lax.dot_general(q, kbuf[slot], _NT, preferred_element_type=F32)
        m = jnp.max(s, axis=-1, keepdims=True)
        p = jnp.exp((s - m) * SCALE)
        pa_s[j % 2] = p.astype(BF16)
        la_s[j % 2] = jnp.broadcast_to(jnp.sum(p, axis=-1, keepdims=True), (B, D))

    def v_phase(i):
        slot = i % NBUF
        b = i // H
        h = i % H
        wait_buf(vbuf.at[slot], kv_sem.at[1, slot])
        o = jnp.dot(pa_s[i % 2], vbuf[slot], preferred_element_type=F32)
        row = lax.broadcasted_iota(jnp.int32, (B, D), 0)
        o = jnp.where(row == b, o / la_s[i % 2], 0.0).astype(BF16)
        acc_a[...] += lax.dot_general(o, head_cols(wot_v, h), _NT,
                                      preferred_element_type=F32)

    wait_buf(xa_v, w_sem.at[0])
    wait_buf(wq_v, w_sem.at[2])
    wait_buf(wot_v, w_sem.at[4])
    acc_a[...] = jnp.zeros(acc_a.shape, F32)
    k_phase(0)

    def b_q(m_lo, m_hi, first):
        def run():
            if first:
                wait_buf(xb_v, w_sem.at[1])
                wait_buf(wqb_v, w_sem.at[3])
            wt = jnp.swapaxes(wqb_v[m_lo:m_hi], 0, 1)
            x = xb_v[:, m_lo:m_hi]
            for h in range(H):
                r = jnp.dot(x, wt[h], preferred_element_type=F32)
                qb_s[h] = r if first else qb_s[h] + r
        return run

    def b_qabs(c_lo, c_hi, first):
        def run():
            if first:
                wait_buf(wuk_v, w_sem.at[6])
            wt = jnp.swapaxes(wuk_v[c_lo:c_hi], 0, 1)
            for h in range(H):
                qa_s[h, :, c_lo:c_hi] = lax.dot_general(
                    qb_s[h].astype(BF16), wt[h], _NT, preferred_element_type=F32)
        return run

    def b_qabs_t():
        qat_s[...] = jnp.swapaxes(qa_s[...], 0, 1).astype(BF16)

    def b_scores(b):
        def run():
            wait_buf(c_v.at[b], w_sem.at[8 + b])
            s = lax.dot_general(qat_s[b], c_v[b], _NT, preferred_element_type=F32)
            m = jnp.max(s, axis=-1, keepdims=True)
            p = jnp.exp((s - m) * SCALE)
            l_s[b] = jnp.broadcast_to(jnp.sum(p, axis=-1, keepdims=True), (H, D))
            p_s[...] = p.astype(BF16)
        return run

    def b_pv(b):
        def run():
            cc = jnp.dot(p_s[...], c_v[b], preferred_element_type=F32)
            cc_s[b] = cc / l_s[b][:, 0:1]
        return run

    def b_ctx(c_lo, c_hi, first):
        def run():
            if first:
                wait_buf(wuv_v, w_sem.at[7])
            wt = jnp.swapaxes(wuv_v[c_lo:c_hi], 0, 1)
            cct = jnp.swapaxes(cc_s[:, :, c_lo:c_hi], 0, 1).astype(BF16)
            for h in range(H):
                r = jnp.dot(cct[h], wt[h], preferred_element_type=F32)
                ctx_s[h] = r if first else ctx_s[h] + r
        return run

    def b_out():
        wait_buf(wobt_v.at[0:n_early], w_sem.at[5])
        o = jnp.zeros((B, M), F32)
        for h in range(n_early):
            o = o + lax.dot_general(ctx_s[h].astype(BF16), wobt_v[h], _NT,
                                    preferred_element_type=F32)
        outb_s[...] = o

    pieces = [b_q(0, 256, True), b_q(256, M, False),
              b_qabs(0, 256, True), b_qabs(256, C, False), b_qabs_t]
    for b in range(B):
        pieces += [b_scores(b), b_pv(b)]
    pieces += [b_ctx(0, 256, True), b_ctx(256, C, False), b_out]

    def step(i, carry):
        @pl.when(i + 1 < NSTEP)
        def _():
            k_phase(i + 1)

        v_phase(i)

        for n, piece in enumerate(pieces):
            pl.when(i == PIECE_START + n * PIECE_STRIDE)(piece)

        @pl.when(i + NBUF < NSTEP)
        def _():
            issue_kv(i + NBUF, i % NBUF)

        pl.when(i + NBUF == NSTEP - 1)(issue_deferred)
        return carry

    lax.fori_loop(0, NSTEP, step, 0)

    out_v[:, 0:M] = acc_a[...].astype(BF16)
    ctx_last = [ctx_s[n_early + j].astype(BF16) for j in range(DEFER)]
    ob = outb_s[...]
    wait_buf(wobt_v.at[n_early:H - 1], d_sem.at[0])
    for j in range(DEFER - 1):
        ob = ob + lax.dot_general(ctx_last[j], wobt_v[n_early + j], _NT,
                                  preferred_element_type=F32)
    wait_buf(wobt_v.at[H - 1], d_sem.at[1])
    ob = ob + lax.dot_general(ctx_last[DEFER - 1], wobt_v[H - 1], _NT,
                              preferred_element_type=F32)
    out_v[:, M:2 * M] = ob.astype(BF16)
    out_copy = copy(out_v, out_hbm, w_sem.at[12])
    out_copy.start()
    out_copy.wait()


@jax.jit
def pallas_concat_heads__mha_block_cached__compressed_kv_cla__decode_kernel(
    A_x: jax.Array,
    A_k_cache: jax.Array,
    A_v_cache: jax.Array,
    A_wq: jax.Array,
    A_wo: jax.Array,
    B_x: jax.Array,
    B_c_kv: jax.Array,
    B_w_q: jax.Array,
    B_w_uk: jax.Array,
    B_w_uv: jax.Array,
    B_w_o: jax.Array,
):
    xa = A_x.reshape(B, M)
    xb = B_x.reshape(B, M)
    wot = A_wo.T
    wobt = B_w_o.transpose(0, 2, 1)

    hbm = pl.BlockSpec(memory_space=pl.ANY)
    scratch = [
        pltpu.VMEM((B, M), BF16),
        pltpu.VMEM((B, M), BF16),
        pltpu.VMEM((M, H * D), BF16),
        pltpu.VMEM((M, H * D), BF16),
        pltpu.VMEM((M, H, D), BF16),
        pltpu.VMEM((C, H, D), BF16),
        pltpu.VMEM((C, H, D), BF16),
        pltpu.VMEM((H, M, D), BF16),
        pltpu.VMEM((B, S, C), BF16),
        pltpu.VMEM((NBUF, S, D), BF16),
        pltpu.VMEM((NBUF, S, D), BF16),
        pltpu.VMEM((B, M), F32),
        pltpu.VMEM((2, B, S), BF16),
        pltpu.VMEM((2, B, D), F32),
        pltpu.VMEM((H, B, D), F32),
        pltpu.VMEM((H, B, C), F32),
        pltpu.VMEM((B, H, C), BF16),
        pltpu.VMEM((H, S), BF16),
        pltpu.VMEM((B, H, D), F32),
        pltpu.VMEM((B, H, C), F32),
        pltpu.VMEM((H, B, D), F32),
        pltpu.VMEM((B, M), F32),
        pltpu.VMEM((B, 2 * M), BF16),
        pltpu.SemaphoreType.DMA((2, NBUF)),
        pltpu.SemaphoreType.DMA((13,)),
        pltpu.SemaphoreType.DMA((2,)),
    ]
    out = pl.pallas_call(
        _kernel,
        out_shape=jax.ShapeDtypeStruct((B, 2 * M), BF16),
        in_specs=[hbm] * 11,
        out_specs=hbm,
        scratch_shapes=scratch,
        compiler_params=pltpu.CompilerParams(
            vmem_limit_bytes=100 * 1024 * 1024,
            disable_semaphore_checks=True,
        ),
    )(xa, A_k_cache, A_v_cache, A_wq, wot, xb, B_c_kv, B_w_q, B_w_uk, B_w_uv, wobt)
    return out.reshape(B, 1, 2 * M)
```

```python
import jax
import jax.numpy as jnp
from jax import lax
from jax.experimental import pallas as pl
from jax.experimental.pallas import tpu as pltpu

B = 4
H = 32
S = 4096
D = 128
M = 576
C = 512
SCALE = D ** -0.5
NSTEP = B * H

KV_CHUNKS = ([192] * 3 + [128] + [192] * 2 + [128] + [192] * 2 + [128] + [192] * 6
             + [128] + [192] * 2 + [128] + [192] * 3)
NBUF = 4
WA_COLS = 2048
W_ROWS = 192
X_CHUNK = 6
C_ROWS = 48
DEFER = 4
PIECE_START = 1
PIECE_STRIDE = 4

BF16 = jnp.bfloat16
F32 = jnp.float32

_NT = (((1,), (1,)), ((), ()))


assert sum(KV_CHUNKS) == S
_KV_SPANS = [(sum(KV_CHUNKS[:j]), n) for j, n in enumerate(KV_CHUNKS)]


def _chunked(total, size, fn):
    n_full = total // size

    def body(c, carry):
        fn(pl.multiple_of(c * size, 8 if size % 8 == 0 else 1), size)
        return carry

    lax.fori_loop(0, n_full, body, 0)
    if total % size:
        fn(n_full * size, total % size)


def _kernel(xa_hbm, k_hbm, v_hbm, wq_hbm, wot_hbm,
            xb_hbm, c_hbm, wqb_hbm, wuk_hbm, wuv_hbm, wobt_hbm,
            out_hbm,
            xa_v, xb_v, wq_v, wot_v, wqb_v, wuk_v, wuv_v, wobt_v, c_v,
            kbuf, vbuf,
            acc_a, pa_s, la_s, qb_s, qa_s, qat_s, p_s, l_s, cc_s, ctx_s, outb_s, out_v,
            kv_sem, w_sem, d_sem):
    copy = pltpu.make_async_copy
    n_sub = M // W_ROWS
    n_early = H - DEFER

    def wait_buf(buf, sem):
        copy(buf, buf, sem).wait()

    def head_cols(ref, h):
        return ref[:, pl.ds(pl.multiple_of(h * D, D), D)]

    def issue_kv(step, slot):
        b = step // H
        h = step % H
        for r0, n in _KV_SPANS:
            copy(v_hbm.at[b, h, pl.ds(r0, n)], vbuf.at[slot, pl.ds(r0, n)],
                 kv_sem.at[1, slot]).start(priority=1)
            copy(k_hbm.at[b, h, pl.ds(r0, n)], kbuf.at[slot, pl.ds(r0, n)],
                 kv_sem.at[0, slot]).start(priority=0)

    copy(xa_hbm, xa_v, w_sem.at[0]).start(priority=0)
    copy(xb_hbm, xb_v, w_sem.at[1]).start(priority=1)

    n_col = (H * D) // WA_COLS

    def wa_body(t, carry):
        idx = (pl.ds(pl.multiple_of((t // n_col) * 8, 8), 8),
               pl.ds(pl.multiple_of((t % n_col) * WA_COLS, D), WA_COLS))
        copy(wq_hbm.at[idx], wq_v.at[idx], w_sem.at[2]).start(priority=0)
        copy(wot_hbm.at[idx], wot_v.at[idx], w_sem.at[4]).start(priority=1)
        return carry

    lax.fori_loop(0, (M // 8) * n_col, wa_body, 0)

    xc = M // (H * n_sub)

    def wqb_chunk(t):
        copy(wqb_hbm.at[pl.ds(t * xc, xc)], wqb_v.at[pl.ds(t * xc, xc)],
             w_sem.at[3]).start(priority=0)

    def wb_body(t, carry):
        wqb_chunk(t)
        h = t // n_sub
        r0 = pl.multiple_of((t % n_sub) * W_ROWS, 8)
        copy(wobt_hbm.at[h, pl.ds(r0, W_ROWS)], wobt_v.at[h, pl.ds(r0, W_ROWS)],
             w_sem.at[5]).start(priority=1)
        return carry

    lax.fori_loop(0, n_early * n_sub, wb_body, 0)

    def wb_tail(t, carry):
        wqb_chunk(t)
        return carry

    lax.fori_loop(n_early * n_sub, H * n_sub, wb_tail, 0)

    def uk_uv(r0, n):
        copy(wuk_hbm.at[pl.ds(r0, n)], wuk_v.at[pl.ds(r0, n)], w_sem.at[6]).start(priority=0)
        copy(wuv_hbm.at[pl.ds(r0, n)], wuv_v.at[pl.ds(r0, n)], w_sem.at[7]).start(priority=1)

    _chunked(C, X_CHUNK, uk_uv)

    for b0 in (0, 2):
        def ckv(r0, n, b0=b0):
            copy(c_hbm.at[b0, pl.ds(r0, n)], c_v.at[b0, pl.ds(r0, n)],
                 w_sem.at[8 + b0]).start(priority=0)
            copy(c_hbm.at[b0 + 1, pl.ds(r0, n)], c_v.at[b0 + 1, pl.ds(r0, n)],
                 w_sem.at[9 + b0]).start(priority=1)

        _chunked(S, C_ROWS, ckv)

    for j in range(NBUF):
        issue_kv(j, j)

    def issue_deferred():
        for j in range(DEFER):
            h = n_early + j
            sem = d_sem.at[0 if j < DEFER - 1 else 1]
            for t in range(n_sub):
                copy(wobt_hbm.at[h, pl.ds(t * W_ROWS, W_ROWS)],
                     wobt_v.at[h, pl.ds(t * W_ROWS, W_ROWS)], sem).start(priority=1)

    def k_phase(j):
        slot = j % NBUF
        h = j % H
        q = jnp.dot(xa_v[...], head_cols(wq_v, h),
                    preferred_element_type=F32).astype(BF16)
        wait_buf(kbuf.at[slot], kv_sem.at[0, slot])
        s = lax.dot_general(q, kbuf[slot], _NT, preferred_element_type=F32)
        m = jnp.max(s, axis=-1, keepdims=True)
        p = jnp.exp((s - m) * SCALE)
        pa_s[j % 2] = p.astype(BF16)
        la_s[j % 2] = jnp.broadcast_to(jnp.sum(p, axis=-1, keepdims=True), (B, D))

    def v_phase(i):
        slot = i % NBUF
        b = i // H
        h = i % H
        wait_buf(vbuf.at[slot], kv_sem.at[1, slot])
        o = jnp.dot(pa_s[i % 2], vbuf[slot], preferred_element_type=F32)
        row = lax.broadcasted_iota(jnp.int32, (B, D), 0)
        o = jnp.where(row == b, o / la_s[i % 2], 0.0).astype(BF16)
        acc_a[...] += lax.dot_general(o, head_cols(wot_v, h), _NT,
                                      preferred_element_type=F32)

    wait_buf(xa_v, w_sem.at[0])
    wait_buf(wq_v, w_sem.at[2])
    wait_buf(wot_v, w_sem.at[4])
    acc_a[...] = jnp.zeros(acc_a.shape, F32)
    k_phase(0)

    def b_q(m_lo, m_hi, first):
        def run():
            if first:
                wait_buf(xb_v, w_sem.at[1])
                wait_buf(wqb_v, w_sem.at[3])
            wt = jnp.swapaxes(wqb_v[m_lo:m_hi], 0, 1)
            x = xb_v[:, m_lo:m_hi]
            for h in range(H):
                r = jnp.dot(x, wt[h], preferred_element_type=F32)
                qb_s[h] = r if first else qb_s[h] + r
        return run

    def b_qabs(c_lo, c_hi, first):
        def run():
            if first:
                wait_buf(wuk_v, w_sem.at[6])
            wt = jnp.swapaxes(wuk_v[c_lo:c_hi], 0, 1)
            for h in range(H):
                qa_s[h, :, c_lo:c_hi] = lax.dot_general(
                    qb_s[h].astype(BF16), wt[h], _NT, preferred_element_type=F32)
        return run

    def b_qabs_t():
        qat_s[...] = jnp.swapaxes(qa_s[...], 0, 1).astype(BF16)

    def b_scores(b):
        def run():
            wait_buf(c_v.at[b], w_sem.at[8 + b])
            s = lax.dot_general(qat_s[b], c_v[b], _NT, preferred_element_type=F32)
            m = jnp.max(s, axis=-1, keepdims=True)
            p = jnp.exp((s - m) * SCALE)
            l_s[b] = jnp.broadcast_to(jnp.sum(p, axis=-1, keepdims=True), (H, D))
            p_s[...] = p.astype(BF16)
        return run

    def b_pv(b):
        def run():
            cc = jnp.dot(p_s[...], c_v[b], preferred_element_type=F32)
            cc_s[b] = cc / l_s[b][:, 0:1]
        return run

    def b_ctx(c_lo, c_hi, first):
        def run():
            if first:
                wait_buf(wuv_v, w_sem.at[7])
            wt = jnp.swapaxes(wuv_v[c_lo:c_hi], 0, 1)
            cct = jnp.swapaxes(cc_s[:, :, c_lo:c_hi], 0, 1).astype(BF16)
            for h in range(H):
                r = jnp.dot(cct[h], wt[h], preferred_element_type=F32)
                ctx_s[h] = r if first else ctx_s[h] + r
        return run

    def b_out():
        wait_buf(wobt_v.at[0:n_early], w_sem.at[5])
        o = jnp.zeros((B, M), F32)
        for h in range(n_early):
            o = o + lax.dot_general(ctx_s[h].astype(BF16), wobt_v[h], _NT,
                                    preferred_element_type=F32)
        outb_s[...] = o

    pieces = [b_q(0, 256, True), b_q(256, M, False),
              b_qabs(0, 256, True), b_qabs(256, C, False), b_qabs_t]
    for b in range(B):
        pieces += [b_scores(b), b_pv(b)]
    pieces += [b_ctx(0, 256, True), b_ctx(256, C, False), b_out]

    def step(i, carry):
        @pl.when(i + 1 < NSTEP)
        def _():
            k_phase(i + 1)

        v_phase(i)

        for n, piece in enumerate(pieces):
            pl.when(i == PIECE_START + n * PIECE_STRIDE)(piece)

        @pl.when(i + NBUF < NSTEP)
        def _():
            issue_kv(i + NBUF, i % NBUF)

        pl.when(i + NBUF == NSTEP - 1)(issue_deferred)
        return carry

    lax.fori_loop(0, NSTEP, step, 0)

    out_v[:, 0:M] = acc_a[...].astype(BF16)
    ctx_last = [ctx_s[n_early + j].astype(BF16) for j in range(DEFER)]
    ob = outb_s[...]
    wait_buf(wobt_v.at[n_early:H - 1], d_sem.at[0])
    for j in range(DEFER - 1):
        ob = ob + lax.dot_general(ctx_last[j], wobt_v[n_early + j], _NT,
                                  preferred_element_type=F32)
    wait_buf(wobt_v.at[H - 1], d_sem.at[1])
    ob = ob + lax.dot_general(ctx_last[DEFER - 1], wobt_v[H - 1], _NT,
                              preferred_element_type=F32)
    out_v[:, M:2 * M] = ob.astype(BF16)
    out_copy = copy(out_v, out_hbm, w_sem.at[12])
    out_copy.start()
    out_copy.wait()


@jax.jit
def pallas_concat_heads__mha_block_cached__compressed_kv_cla__decode_kernel(
    A_x: jax.Array,
    A_k_cache: jax.Array,
    A_v_cache: jax.Array,
    A_wq: jax.Array,
    A_wo: jax.Array,
    B_x: jax.Array,
    B_c_kv: jax.Array,
    B_w_q: jax.Array,
    B_w_uk: jax.Array,
    B_w_uv: jax.Array,
    B_w_o: jax.Array,
):
    xa = A_x.reshape(B, M)
    xb = B_x.reshape(B, M)
    wot = A_wo.T
    wobt = B_w_o.transpose(0, 2, 1)

    hbm = pl.BlockSpec(memory_space=pl.ANY)
    scratch = [
        pltpu.VMEM((B, M), BF16),
        pltpu.VMEM((B, M), BF16),
        pltpu.VMEM((M, H * D), BF16),
        pltpu.VMEM((M, H * D), BF16),
        pltpu.VMEM((M, H, D), BF16),
        pltpu.VMEM((C, H, D), BF16),
        pltpu.VMEM((C, H, D), BF16),
        pltpu.VMEM((H, M, D), BF16),
        pltpu.VMEM((B, S, C), BF16),
        pltpu.VMEM((NBUF, S, D), BF16),
        pltpu.VMEM((NBUF, S, D), BF16),
        pltpu.VMEM((B, M), F32),
        pltpu.VMEM((2, B, S), BF16),
        pltpu.VMEM((2, B, D), F32),
        pltpu.VMEM((H, B, D), F32),
        pltpu.VMEM((H, B, C), F32),
        pltpu.VMEM((B, H, C), BF16),
        pltpu.VMEM((H, S), BF16),
        pltpu.VMEM((B, H, D), F32),
        pltpu.VMEM((B, H, C), F32),
        pltpu.VMEM((H, B, D), F32),
        pltpu.VMEM((B, M), F32),
        pltpu.VMEM((B, 2 * M), BF16),
        pltpu.SemaphoreType.DMA((2, NBUF)),
        pltpu.SemaphoreType.DMA((13,)),
        pltpu.SemaphoreType.DMA((2,)),
    ]
    out = pl.pallas_call(
        _kernel,
        out_shape=jax.ShapeDtypeStruct((B, 2 * M), BF16),
        in_specs=[hbm] * 11,
        out_specs=hbm,
        scratch_shapes=scratch,
        compiler_params=pltpu.CompilerParams(
            vmem_limit_bytes=100 * 1024 * 1024,
            disable_semaphore_checks=True,
        ),
    )(xa, A_k_cache, A_v_cache, A_wq, wot, xb, B_c_kv, B_w_q, B_w_uk, B_w_uv, wobt)
    return out.reshape(B, 1, 2 * M)
```

```python
import jax
import jax.numpy as jnp
from jax import lax
from jax.experimental import pallas as pl
from jax.experimental.pallas import tpu as pltpu

B = 4
H = 32
S = 4096
D = 128
M = 576
C = 512
SCALE = D ** -0.5
NSTEP = B * H

KV_CHUNKS = ([192] * 3 + [128] + [192] * 2 + [128] + [192] * 2 + [128] + [192] * 6
             + [128] + [192] * 2 + [128] + [192] * 3)
NBUF = 4
WA_COLS = 2048
W_ROWS = 192
X_CHUNK = 6
C_RUNS = [(48, 3), (32, 1), (48, 10), (32, 1), (48, 7)] * 4
DEFER = 4
PIECE_START = 1
PIECE_STRIDE = 4

BF16 = jnp.bfloat16
F32 = jnp.float32

_NT = (((1,), (1,)), ((), ()))


assert sum(KV_CHUNKS) == S
_KV_SPANS = [(sum(KV_CHUNKS[:j]), n) for j, n in enumerate(KV_CHUNKS)]


def _chunked(total, size, fn):
    n_full = total // size

    def body(c, carry):
        fn(pl.multiple_of(c * size, 8 if size % 8 == 0 else 1), size)
        return carry

    lax.fori_loop(0, n_full, body, 0)
    if total % size:
        fn(n_full * size, total % size)


def _runs(runs, fn):
    start = 0
    for size, count in runs:
        if count == 1:
            fn(start, size)
        else:
            def body(c, carry, start=start, size=size):
                fn(pl.multiple_of(start + c * size, 8), size)
                return carry

            lax.fori_loop(0, count, body, 0)
        start += size * count
    return start


def _kernel(xa_hbm, k_hbm, v_hbm, wq_hbm, wot_hbm,
            xb_hbm, c_hbm, wqb_hbm, wuk_hbm, wuv_hbm, wobt_hbm,
            out_hbm,
            xa_v, xb_v, wq_v, wot_v, wqb_v, wuk_v, wuv_v, wobt_v, c_v,
            kbuf, vbuf,
            acc_a, pa_s, la_s, qb_s, qa_s, qat_s, p_s, l_s, cc_s, ctx_s, outb_s, out_v,
            kv_sem, w_sem, d_sem):
    copy = pltpu.make_async_copy
    n_sub = M // W_ROWS
    n_early = H - DEFER

    def wait_buf(buf, sem):
        copy(buf, buf, sem).wait()

    def head_cols(ref, h):
        return ref[:, pl.ds(pl.multiple_of(h * D, D), D)]

    def issue_kv(step, slot):
        b = step // H
        h = step % H
        for r0, n in _KV_SPANS:
            copy(v_hbm.at[b, h, pl.ds(r0, n)], vbuf.at[slot, pl.ds(r0, n)],
                 kv_sem.at[1, slot]).start(priority=1)
            copy(k_hbm.at[b, h, pl.ds(r0, n)], kbuf.at[slot, pl.ds(r0, n)],
                 kv_sem.at[0, slot]).start(priority=0)

    copy(xa_hbm, xa_v, w_sem.at[0]).start(priority=0)
    copy(xb_hbm, xb_v, w_sem.at[1]).start(priority=1)

    n_col = (H * D) // WA_COLS

    def wa_body(t, carry):
        idx = (pl.ds(pl.multiple_of((t // n_col) * 8, 8), 8),
               pl.ds(pl.multiple_of((t % n_col) * WA_COLS, D), WA_COLS))
        copy(wot_hbm.at[idx], wot_v.at[idx], w_sem.at[4]).start(priority=1)
        copy(wq_hbm.at[idx], wq_v.at[idx], w_sem.at[2]).start(priority=0)
        return carry

    lax.fori_loop(0, (M // 8) * n_col, wa_body, 0)

    xc = M // (H * n_sub)

    def wqb_chunk(t):
        copy(wqb_hbm.at[pl.ds(t * xc, xc)], wqb_v.at[pl.ds(t * xc, xc)],
             w_sem.at[3]).start(priority=0)

    def wb_body(t, carry):
        h = t // n_sub
        r0 = pl.multiple_of((t % n_sub) * W_ROWS, 8)
        copy(wobt_hbm.at[h, pl.ds(r0, W_ROWS)], wobt_v.at[h, pl.ds(r0, W_ROWS)],
             w_sem.at[5]).start(priority=1)
        wqb_chunk(t)
        return carry

    lax.fori_loop(0, n_early * n_sub, wb_body, 0)

    def wb_tail(t, carry):
        wqb_chunk(t)
        return carry

    lax.fori_loop(n_early * n_sub, H * n_sub, wb_tail, 0)

    def uk_uv(r0, n):
        copy(wuv_hbm.at[pl.ds(r0, n)], wuv_v.at[pl.ds(r0, n)], w_sem.at[7]).start(priority=1)
        copy(wuk_hbm.at[pl.ds(r0, n)], wuk_v.at[pl.ds(r0, n)], w_sem.at[6]).start(priority=0)

    _chunked(C, X_CHUNK, uk_uv)

    for b0 in (0, 2):
        def ckv(r0, n, b0=b0):
            copy(c_hbm.at[b0 + 1, pl.ds(r0, n)], c_v.at[b0 + 1, pl.ds(r0, n)],
                 w_sem.at[9 + b0]).start(priority=1)
            copy(c_hbm.at[b0, pl.ds(r0, n)], c_v.at[b0, pl.ds(r0, n)],
                 w_sem.at[8 + b0]).start(priority=0)

        assert _runs(C_RUNS, ckv) == S

    for j in range(NBUF):
        issue_kv(j, j)

    def issue_deferred():
        for j in range(DEFER):
            h = n_early + j
            sem = d_sem.at[0 if j < DEFER - 1 else 1]
            for t in range(n_sub):
                copy(wobt_hbm.at[h, pl.ds(t * W_ROWS, W_ROWS)],
                     wobt_v.at[h, pl.ds(t * W_ROWS, W_ROWS)], sem).start(priority=1)

    def k_phase(j):
        slot = j % NBUF
        h = j % H
        q = jnp.dot(xa_v[...], head_cols(wq_v, h),
                    preferred_element_type=F32).astype(BF16)
        wait_buf(kbuf.at[slot], kv_sem.at[0, slot])
        s = lax.dot_general(q, kbuf[slot], _NT, preferred_element_type=F32)
        m = jnp.max(s, axis=-1, keepdims=True)
        p = jnp.exp((s - m) * SCALE)
        pa_s[j % 2] = p.astype(BF16)
        la_s[j % 2] = jnp.broadcast_to(jnp.sum(p, axis=-1, keepdims=True), (B, D))

    def v_phase(i):
        slot = i % NBUF
        b = i // H
        h = i % H
        wait_buf(vbuf.at[slot], kv_sem.at[1, slot])
        o = jnp.dot(pa_s[i % 2], vbuf[slot], preferred_element_type=F32)
        row = lax.broadcasted_iota(jnp.int32, (B, D), 0)
        o = jnp.where(row == b, o / la_s[i % 2], 0.0).astype(BF16)
        acc_a[...] += lax.dot_general(o, head_cols(wot_v, h), _NT,
                                      preferred_element_type=F32)

    wait_buf(xa_v, w_sem.at[0])
    wait_buf(wq_v, w_sem.at[2])
    wait_buf(wot_v, w_sem.at[4])
    acc_a[...] = jnp.zeros(acc_a.shape, F32)
    k_phase(0)

    def b_q(m_lo, m_hi, first):
        def run():
            if first:
                wait_buf(xb_v, w_sem.at[1])
                wait_buf(wqb_v, w_sem.at[3])
            wt = jnp.swapaxes(wqb_v[m_lo:m_hi], 0, 1)
            x = xb_v[:, m_lo:m_hi]
            for h in range(H):
                r = jnp.dot(x, wt[h], preferred_element_type=F32)
                qb_s[h] = r if first else qb_s[h] + r
        return run

    def b_qabs(c_lo, c_hi, first):
        def run():
            if first:
                wait_buf(wuk_v, w_sem.at[6])
            wt = jnp.swapaxes(wuk_v[c_lo:c_hi], 0, 1)
            for h in range(H):
                qa_s[h, :, c_lo:c_hi] = lax.dot_general(
                    qb_s[h].astype(BF16), wt[h], _NT, preferred_element_type=F32)
        return run

    def b_qabs_t():
        qat_s[...] = jnp.swapaxes(qa_s[...], 0, 1).astype(BF16)

    def b_scores(b):
        def run():
            wait_buf(c_v.at[b], w_sem.at[8 + b])
            s = lax.dot_general(qat_s[b], c_v[b], _NT, preferred_element_type=F32)
            m = jnp.max(s, axis=-1, keepdims=True)
            p = jnp.exp((s - m) * SCALE)
            l_s[b] = jnp.broadcast_to(jnp.sum(p, axis=-1, keepdims=True), (H, D))
            p_s[...] = p.astype(BF16)
        return run

    def b_pv(b):
        def run():
            cc = jnp.dot(p_s[...], c_v[b], preferred_element_type=F32)
            cc_s[b] = cc / l_s[b][:, 0:1]
        return run

    def b_ctx(c_lo, c_hi, first):
        def run():
            if first:
                wait_buf(wuv_v, w_sem.at[7])
            wt = jnp.swapaxes(wuv_v[c_lo:c_hi], 0, 1)
            cct = jnp.swapaxes(cc_s[:, :, c_lo:c_hi], 0, 1).astype(BF16)
            for h in range(H):
                r = jnp.dot(cct[h], wt[h], preferred_element_type=F32)
                ctx_s[h] = r if first else ctx_s[h] + r
        return run

    def b_out():
        wait_buf(wobt_v.at[0:n_early], w_sem.at[5])
        o = jnp.zeros((B, M), F32)
        for h in range(n_early):
            o = o + lax.dot_general(ctx_s[h].astype(BF16), wobt_v[h], _NT,
                                    preferred_element_type=F32)
        outb_s[...] = o

    pieces = [b_q(0, 256, True), b_q(256, M, False),
              b_qabs(0, 256, True), b_qabs(256, C, False), b_qabs_t]
    for b in range(B):
        pieces += [b_scores(b), b_pv(b)]
    pieces += [b_ctx(0, 256, True), b_ctx(256, C, False), b_out]

    def step(i, carry):
        @pl.when(i + 1 < NSTEP)
        def _():
            k_phase(i + 1)

        v_phase(i)

        for n, piece in enumerate(pieces):
            pl.when(i == PIECE_START + n * PIECE_STRIDE)(piece)

        @pl.when(i + NBUF < NSTEP)
        def _():
            issue_kv(i + NBUF, i % NBUF)

        pl.when(i + NBUF == NSTEP - 1)(issue_deferred)
        return carry

    lax.fori_loop(0, NSTEP, step, 0)

    out_v[:, 0:M] = acc_a[...].astype(BF16)
    ctx_last = [ctx_s[n_early + j].astype(BF16) for j in range(DEFER)]
    ob = outb_s[...]
    wait_buf(wobt_v.at[n_early:H - 1], d_sem.at[0])
    for j in range(DEFER - 1):
        ob = ob + lax.dot_general(ctx_last[j], wobt_v[n_early + j], _NT,
                                  preferred_element_type=F32)
    wait_buf(wobt_v.at[H - 1], d_sem.at[1])
    ob = ob + lax.dot_general(ctx_last[DEFER - 1], wobt_v[H - 1], _NT,
                              preferred_element_type=F32)
    out_v[:, M:2 * M] = ob.astype(BF16)
    out_copy = copy(out_v, out_hbm, w_sem.at[12])
    out_copy.start()
    out_copy.wait()


@jax.jit
def pallas_concat_heads__mha_block_cached__compressed_kv_cla__decode_kernel(
    A_x: jax.Array,
    A_k_cache: jax.Array,
    A_v_cache: jax.Array,
    A_wq: jax.Array,
    A_wo: jax.Array,
    B_x: jax.Array,
    B_c_kv: jax.Array,
    B_w_q: jax.Array,
    B_w_uk: jax.Array,
    B_w_uv: jax.Array,
    B_w_o: jax.Array,
):
    xa = A_x.reshape(B, M)
    xb = B_x.reshape(B, M)
    wot = A_wo.T
    wobt = B_w_o.transpose(0, 2, 1)

    hbm = pl.BlockSpec(memory_space=pl.ANY)
    scratch = [
        pltpu.VMEM((B, M), BF16),
        pltpu.VMEM((B, M), BF16),
        pltpu.VMEM((M, H * D), BF16),
        pltpu.VMEM((M, H * D), BF16),
        pltpu.VMEM((M, H, D), BF16),
        pltpu.VMEM((C, H, D), BF16),
        pltpu.VMEM((C, H, D), BF16),
        pltpu.VMEM((H, M, D), BF16),
        pltpu.VMEM((B, S, C), BF16),
        pltpu.VMEM((NBUF, S, D), BF16),
        pltpu.VMEM((NBUF, S, D), BF16),
        pltpu.VMEM((B, M), F32),
        pltpu.VMEM((2, B, S), BF16),
        pltpu.VMEM((2, B, D), F32),
        pltpu.VMEM((H, B, D), F32),
        pltpu.VMEM((H, B, C), F32),
        pltpu.VMEM((B, H, C), BF16),
        pltpu.VMEM((H, S), BF16),
        pltpu.VMEM((B, H, D), F32),
        pltpu.VMEM((B, H, C), F32),
        pltpu.VMEM((H, B, D), F32),
        pltpu.VMEM((B, M), F32),
        pltpu.VMEM((B, 2 * M), BF16),
        pltpu.SemaphoreType.DMA((2, NBUF)),
        pltpu.SemaphoreType.DMA((13,)),
        pltpu.SemaphoreType.DMA((2,)),
    ]
    out = pl.pallas_call(
        _kernel,
        out_shape=jax.ShapeDtypeStruct((B, 2 * M), BF16),
        in_specs=[hbm] * 11,
        out_specs=hbm,
        scratch_shapes=scratch,
        compiler_params=pltpu.CompilerParams(
            vmem_limit_bytes=100 * 1024 * 1024,
            disable_semaphore_checks=True,
        ),
    )(xa, A_k_cache, A_v_cache, A_wq, wot, xb, B_c_kv, B_w_q, B_w_uk, B_w_uv, wobt)
    return out.reshape(B, 1, 2 * M)
```
